```python
import os as _os
_os.environ.setdefault("JAX_PLATFORMS", "cpu")
import jax
import jax.numpy as jnp

def _softmax(x, axis=-1):
    return jax.nn.softmax(x, axis=axis)
def _gelu(x):
    return jax.nn.gelu(x, approximate=True)
def _silu(x):
    return jax.nn.silu(x)
def _sigmoid(x):
    return jax.nn.sigmoid(x)
def _layernorm(x, axis=-1, eps=1e-5):
    m = jnp.mean(x, axis=axis, keepdims=True)
    v = jnp.var(x, axis=axis, keepdims=True)
    return (x - m) / jnp.sqrt(v + eps)
def _scatter_add(tgt, idx, src, axis=0):
    return tgt.at[idx].add(src)
def _segment_sum(src, seg, n):
    return jax.ops.segment_sum(src, seg, n)
class _Rng:
    def __init__(self, key):
        self._k = key
    def _next(self):
        self._k, sub = jax.random.split(self._k)
        return sub
    def normal(self, shape):
        return jax.random.normal(self._next(), shape, dtype=jnp.bfloat16)
    def randint(self, lo, hi, shape):
        return jax.random.randint(self._next(), shape, lo, hi, dtype=jnp.int32)
    def uniform(self, shape, lo=0.0, hi=1.0):
        return jax.random.uniform(self._next(), shape, jnp.bfloat16, lo, hi)
    def permutation(self, n):
        return jax.random.permutation(self._next(), n)


kernel_name = 'standalone__mha_softmax__near_ridge'

def setup_inputs():
    _rng = _Rng(jax.random.key(int.from_bytes(__import__("os").urandom(4), "little")))
    _w = (lambda a: (lambda t: t.astype(jnp.bfloat16) if jnp.issubdtype(t.dtype, jnp.floating) else t)(jnp.asarray(a)))
    B, H, Sq, Sk, D = 8, 32, 304, 2048, 128
    return {
        "q": _w((lambda *s: _rng.normal(s) * 0.4)(B, H, Sq, D)),
        "k": _w((lambda *s: _rng.normal(s) * 0.4)(B, H, Sk, D)),
        "v": _w((lambda *s: _rng.normal(s) * 0.05)(B, H, Sk, D)),
    }

def reference(q, k, v):
    scale = q.shape[-1] ** -0.5
    scores = jnp.einsum("bhqd,bhkd->bhqk", q, k) * scale
    p = _softmax(scores, axis=-1)
    return jnp.einsum("bhqk,bhkd->bhqd", p, v)
```

```python
import jax
import jax.numpy as jnp
from jax import lax
from jax.experimental import pallas as pl
from jax.experimental.pallas import tpu as pltpu

LOG2E = 1.4426950408889634
QK_CONTRACT = (((1,), (1,)), ((), ()))

GROUP = 16
WBATCH = 4
VMEM_LIMIT = 100 * 1024 * 1024


def _load_bf16(ref):
  return pltpu.bitcast(ref.bitcast(jnp.int32)[...], jnp.bfloat16)


def _kernel(q_hbm, k_hbm, v_hbm, o_hbm, *scratch):
  n_obuf = GROUP // WBATCH
  qbuf = scratch[0:GROUP]
  kbuf = scratch[GROUP:2 * GROUP]
  vbuf = scratch[2 * GROUP:3 * GROUP]
  obuf = scratch[3 * GROUP:3 * GROUP + n_obuf]
  sems, osems = scratch[3 * GROUP + n_obuf:]

  nheads = q_hbm.shape[0]
  niters = nheads // GROUP
  scale = LOG2E * (q_hbm.shape[-1] ** -0.5)

  def copy_q(h, s):
    return pltpu.make_async_copy(q_hbm.at[h], qbuf[s], sems.at[0, s])

  def copy_k(h, s):
    return pltpu.make_async_copy(k_hbm.at[h], kbuf[s], sems.at[1, s])

  def copy_v(h, s):
    return pltpu.make_async_copy(v_hbm.at[h], vbuf[s], sems.at[2, s])

  def copy_o(t, j):
    return pltpu.make_async_copy(
        obuf[j], o_hbm.at[pl.ds(t * GROUP + j * WBATCH, WBATCH)], osems.at[j])

  def scores(s):
    qk = lax.dot_general(_load_bf16(qbuf[s]), _load_bf16(kbuf[s]), QK_CONTRACT,
                         preferred_element_type=jnp.float32)
    return (qk - jnp.max(qk, axis=-1, keepdims=True)) * scale

  def attend(shifted, s):
    p = jnp.exp2(shifted)
    denom = jnp.sum(p, axis=-1, keepdims=True)
    acc = jnp.dot(p.astype(jnp.bfloat16), _load_bf16(vbuf[s]),
                  preferred_element_type=jnp.float32)
    inv = pl.reciprocal(denom, approx=True)
    inv = inv * (2.0 - denom * inv)
    obuf[s // WBATCH][s % WBATCH] = (acc * inv).astype(o_hbm.dtype)

  for s in range(GROUP):
    copy_q(s, s).start()
    copy_k(s, s).start()
    copy_v(s, s).start()
  copy_q(0, 0).wait()
  copy_k(0, 0).wait()

  def body(t, carry):
    for s in range(GROUP):
      head = t * GROUP + s
      shifted = scores(s)

      copy_v(head, s).wait()
      nxt = (s + 1) % GROUP

      @pl.when(head + 1 < nheads)
      def _():
        copy_q(head + 1, nxt).wait()
        copy_k(head + 1, nxt).wait()

      if s % WBATCH == 0:
        @pl.when(t > 0)
        def _():
          copy_o(t - 1, s // WBATCH).wait()

      @pl.when(head + GROUP < nheads)
      def _():
        copy_q(head + GROUP, s).start()
        copy_k(head + GROUP, s).start()

      attend(shifted, s)

      if s % WBATCH == WBATCH - 1:
        copy_o(t, s // WBATCH).start()

      @pl.when(head + GROUP < nheads)
      def _():
        copy_v(head + GROUP, s).start()

    return carry

  lax.fori_loop(0, niters, body, 0)
  for j in range(n_obuf):
    copy_o(niters - 1, j).wait()


@jax.jit
def pallas_standalone__mha_softmax__near_ridge_kernel(
    q: jax.Array,
    k: jax.Array,
    v: jax.Array,
):
  batch, heads, seq_q, dim = q.shape
  seq_k = k.shape[2]
  nheads = batch * heads

  q3 = q.reshape(nheads, seq_q, dim)
  k3 = k.reshape(nheads, seq_k, dim)
  v3 = v.reshape(nheads, seq_k, dim)

  scratch = (
      [pltpu.VMEM((seq_q, dim), q.dtype)] * GROUP
      + [pltpu.VMEM((seq_k, dim), k.dtype)] * GROUP
      + [pltpu.VMEM((seq_k, dim), v.dtype)] * GROUP
      + [pltpu.VMEM((WBATCH, seq_q, dim), q.dtype)] * (GROUP // WBATCH)
      + [pltpu.SemaphoreType.DMA((3, GROUP)),
         pltpu.SemaphoreType.DMA((GROUP // WBATCH,))])

  out = pl.pallas_call(
      _kernel,
      in_specs=[pl.BlockSpec(memory_space=pl.ANY)] * 3,
      out_specs=pl.BlockSpec(memory_space=pl.ANY),
      out_shape=jax.ShapeDtypeStruct((nheads, seq_q, dim), q.dtype),
      scratch_shapes=scratch,
      compiler_params=pltpu.CompilerParams(
          vmem_limit_bytes=VMEM_LIMIT,
          disable_bounds_checks=True,
          flags={"XLA_TPU_RESCHEDULE_DMA_DONES": True},
      ),
  )(q3, k3, v3)

  return out.reshape(batch, heads, seq_q, dim)
```

```python
import jax
import jax.numpy as jnp
from jax import lax
from jax.experimental import pallas as pl
from jax.experimental.pallas import tpu as pltpu

LOG2E = 1.4426950408889634
QK_CONTRACT = (((1,), (1,)), ((), ()))

GROUP = 16
WBATCH = 4
ROUNDS = 4
TIE_LAG = 2
VMEM_LIMIT = 100 * 1024 * 1024


def _load_bf16(ref):
  return pltpu.bitcast(ref.bitcast(jnp.int32)[...], jnp.bfloat16)


def _after(value, marker_bits, marker):
  return jnp.where(marker_bits != 0, value, marker)


def _kernel(q_hbm, k_hbm, v_hbm, o_hbm, *scratch):
  n_obuf = GROUP // WBATCH
  qbuf = scratch[0:GROUP]
  kbuf = scratch[GROUP:2 * GROUP]
  vbuf = scratch[2 * GROUP:3 * GROUP]
  obuf = scratch[3 * GROUP:3 * GROUP + n_obuf]
  sems, osems = scratch[3 * GROUP + n_obuf:]

  nheads = q_hbm.shape[0]
  niters = nheads // GROUP
  scale = LOG2E * (q_hbm.shape[-1] ** -0.5)

  def copy_q(h, s):
    return pltpu.make_async_copy(q_hbm.at[h], qbuf[s], sems.at[0, s])

  def copy_k(h, s):
    return pltpu.make_async_copy(k_hbm.at[h], kbuf[s], sems.at[1, s])

  def copy_v(h, s):
    return pltpu.make_async_copy(v_hbm.at[h], vbuf[s], sems.at[2, s])

  def copy_o(t, j):
    return pltpu.make_async_copy(
        obuf[j], o_hbm.at[pl.ds(t * GROUP + j * WBATCH, WBATCH)], osems.at[j])

  def scores(s):
    qk = lax.dot_general(_load_bf16(qbuf[s]), _load_bf16(kbuf[s]), QK_CONTRACT,
                         preferred_element_type=jnp.float32)
    return qk, jnp.max(qk, axis=-1, keepdims=True)

  def store_normalized(acc, denom, s):
    inv = pl.reciprocal(denom, approx=True)
    inv = inv * (2.0 - denom * inv)
    obuf[s // WBATCH][s % WBATCH] = (acc * inv).astype(o_hbm.dtype)

  def attend(qk, row_max, s):
    p = jnp.exp2((qk - row_max) * scale)
    acc = jnp.dot(p.astype(jnp.bfloat16), _load_bf16(vbuf[s]),
                  preferred_element_type=jnp.float32)
    denom = jnp.sum(p, axis=-1, keepdims=True)
    store_normalized(acc, denom, s)
    return denom

  def attend_in_rounds(qk, row_max, s):
    width = qk.shape[1] // ROUNDS
    v32 = vbuf[s].bitcast(jnp.int32)
    acc = lane_sums = prev = None
    for r in range(ROUNDS):
      shift = row_max
      if prev is not None:
        bits = lax.bitcast_convert_type(prev, jnp.int32) | 1
        shift = _after(jnp.broadcast_to(row_max, prev.shape), bits, prev)
        shift = jnp.concatenate([shift] * (width // 128), axis=1)
      p = jnp.exp2((qk[:, r * width:(r + 1) * width] - shift) * scale)
      v = pltpu.bitcast(v32[r * width // 2:(r + 1) * width // 2, :], jnp.bfloat16)
      prev = jnp.dot(p.astype(jnp.bfloat16), v, preferred_element_type=jnp.float32)
      acc = prev if acc is None else acc + prev
      part = p[:, 0:128]
      for j in range(1, width // 128):
        part = part + p[:, 128 * j:128 * (j + 1)]
      lane_sums = part if lane_sums is None else lane_sums + part
    store_normalized(acc, jnp.sum(lane_sums, axis=-1, keepdims=True), s)

  for s in range(GROUP):
    copy_q(s, s).start()
    copy_k(s, s).start()
    copy_v(s, s).start()
  copy_q(0, 0).wait()
  copy_k(0, 0).wait()

  def body(t, carry):
    denoms = {}
    for s in range(GROUP):
      head = t * GROUP + s
      qk, row_max = scores(s)

      copy_v(head, s).wait()
      nxt = (s + 1) % GROUP

      @pl.when(head + 1 < nheads)
      def _():
        copy_q(head + 1, nxt).wait()
        copy_k(head + 1, nxt).wait()

      if s % WBATCH == 0:
        @pl.when(t > 0)
        def _():
          copy_o(t - 1, s // WBATCH).wait()

      @pl.when(head + GROUP < nheads)
      def _():
        copy_q(head + GROUP, s).start()
        copy_k(head + GROUP, s).start()

      if s >= TIE_LAG:
        due = denoms[s - TIE_LAG]
        row_max = _after(row_max, lax.bitcast_convert_type(due, jnp.int32), due)
      if s == GROUP - 1:
        attend_in_rounds(qk, row_max, s)
      else:
        denoms[s] = attend(qk, row_max, s)

      if s % WBATCH == WBATCH - 1:
        copy_o(t, s // WBATCH).start()

      @pl.when(head + GROUP < nheads)
      def _():
        copy_v(head + GROUP, s).start()

    return carry

  lax.fori_loop(0, niters, body, 0)
  for j in range(n_obuf):
    copy_o(niters - 1, j).wait()


@jax.jit
def pallas_standalone__mha_softmax__near_ridge_kernel(
    q: jax.Array,
    k: jax.Array,
    v: jax.Array,
):
  batch, heads, seq_q, dim = q.shape
  seq_k = k.shape[2]
  nheads = batch * heads

  q3 = q.reshape(nheads, seq_q, dim)
  k3 = k.reshape(nheads, seq_k, dim)
  v3 = v.reshape(nheads, seq_k, dim)

  scratch = (
      [pltpu.VMEM((seq_q, dim), q.dtype)] * GROUP
      + [pltpu.VMEM((seq_k, dim), k.dtype)] * GROUP
      + [pltpu.VMEM((seq_k, dim), v.dtype)] * GROUP
      + [pltpu.VMEM((WBATCH, seq_q, dim), q.dtype)] * (GROUP // WBATCH)
      + [pltpu.SemaphoreType.DMA((3, GROUP)),
         pltpu.SemaphoreType.DMA((GROUP // WBATCH,))])

  out = pl.pallas_call(
      _kernel,
      in_specs=[pl.BlockSpec(memory_space=pl.ANY)] * 3,
      out_specs=pl.BlockSpec(memory_space=pl.ANY),
      out_shape=jax.ShapeDtypeStruct((nheads, seq_q, dim), q.dtype),
      scratch_shapes=scratch,
      compiler_params=pltpu.CompilerParams(
          vmem_limit_bytes=VMEM_LIMIT,
          disable_bounds_checks=True,
          disable_semaphore_checks=True,
          flags={"XLA_TPU_RESCHEDULE_DMA_DONES": True},
      ),
  )(q3, k3, v3)

  return out.reshape(batch, heads, seq_q, dim)
```

```python
import jax
import jax.numpy as jnp
from jax import lax
from jax.experimental import pallas as pl
from jax.experimental.pallas import tpu as pltpu

LOG2E = 1.4426950408889634
QK_CONTRACT = (((1,), (1,)), ((), ()))

GROUP = 23
WBATCH = 4
ROUNDS = 4
TIE_LAG = 2
VMEM_LIMIT = 64 * 1024 * 1024


def _bits(ref):
  return ref.bitcast(jnp.int32)


def _as_bf16(words):
  return pltpu.bitcast(words, jnp.bfloat16)


def _after(value, marker_bits, marker):
  return jnp.where(marker_bits != 0, value, marker)


def _when(condition):
  if isinstance(condition, bool):
    return lambda f: f() if condition else None
  return pl.when(condition)


def _kernel(q_hbm, k_hbm, v_hbm, o_hbm, *scratch):
  nheads, _, dim = q_hbm.shape
  seq_k = k_hbm.shape[1]
  niters, leftover = divmod(nheads, GROUP)
  n_obuf = -(-GROUP // WBATCH)
  full_sizes = [min(WBATCH, GROUP - j * WBATCH) for j in range(n_obuf)]
  scale = LOG2E * (dim ** -0.5)

  qbuf = scratch[0:GROUP]
  kbuf = scratch[GROUP:2 * GROUP]
  vbuf = scratch[2 * GROUP:3 * GROUP]
  obuf = scratch[3 * GROUP:3 * GROUP + n_obuf]
  sems, osems = scratch[3 * GROUP + n_obuf:]

  def copy_q(h, s):
    return pltpu.make_async_copy(q_hbm.at[h], qbuf[s], sems.at[0, s])

  def copy_k(h, s):
    return pltpu.make_async_copy(k_hbm.at[h], kbuf[s], sems.at[1, s])

  def copy_v(h, s):
    return pltpu.make_async_copy(v_hbm.at[h], vbuf[s], sems.at[2, s])

  def copy_o(base, j, n):
    return pltpu.make_async_copy(
        obuf[j].at[pl.ds(0, n)], o_hbm.at[pl.ds(base + j * WBATCH, n)], osems.at[j])

  def copy_o_head(base, j, i):
    return pltpu.make_async_copy(
        obuf[j].at[i], o_hbm.at[base + j * WBATCH + i], osems.at[j])

  def scores(s):
    qk = lax.dot_general(_as_bf16(_bits(qbuf[s])[...]), _as_bf16(_bits(kbuf[s])[...]),
                         QK_CONTRACT, preferred_element_type=jnp.float32)
    return qk, jnp.max(qk, axis=-1, keepdims=True)

  def store_normalized(acc, denom, s):
    inv = pl.reciprocal(denom, approx=True)
    inv = inv * (2.0 - denom * inv)
    obuf[s // WBATCH][s % WBATCH] = (acc * inv).astype(o_hbm.dtype)

  def attend(qk, row_max, s):
    p = jnp.exp2((qk - row_max) * scale)
    acc = jnp.dot(p.astype(jnp.bfloat16), _as_bf16(_bits(vbuf[s])[...]),
                  preferred_element_type=jnp.float32)
    denom = jnp.sum(p, axis=-1, keepdims=True)
    store_normalized(acc, denom, s)
    return denom

  def attend_in_rounds(qk, row_max, s):
    width = seq_k // ROUNDS
    acc = lane_sums = part_acc = part_sum = None
    for r in range(ROUNDS):
      shift = row_max
      if r > 0:
        marker = (lax.bitcast_convert_type(part_acc, jnp.int32)
                  | lax.bitcast_convert_type(part_sum, jnp.int32) | 1)
        shift = _after(jnp.broadcast_to(row_max, part_acc.shape), marker, part_acc)
        shift = jnp.concatenate([shift] * (width // 128), axis=1)
      p = jnp.exp2((qk[:, r * width:(r + 1) * width] - shift) * scale)
      v = _as_bf16(_bits(vbuf[s])[r * width // 2:(r + 1) * width // 2, :])
      part_acc = jnp.dot(p.astype(jnp.bfloat16), v, preferred_element_type=jnp.float32)
      part_sum = p[:, 0:128]
      for j in range(1, width // 128):
        part_sum = part_sum + p[:, 128 * j:128 * (j + 1)]
      acc = part_acc if acc is None else acc + part_acc
      lane_sums = part_sum if lane_sums is None else lane_sums + part_sum
    store_normalized(acc, jnp.sum(lane_sums, axis=-1, keepdims=True), s)

  def run_heads(base, count, final):
    n_batches = -(-count // WBATCH)
    denoms = {}
    for s in range(count):
      head = base + s
      batch, pos = divmod(s, WBATCH)
      qk, row_max = scores(s)

      @_when(head + GROUP < nheads)
      def _():
        copy_q(head + GROUP, s).start()
        copy_k(head + GROUP, s).start()

      copy_v(head, s).wait()

      if pos == 0:
        @_when(base >= GROUP)
        def _():
          copy_o(base - GROUP, batch, full_sizes[batch]).wait()

      if s >= TIE_LAG:
        due = denoms[s - TIE_LAG]
        row_max = _after(row_max, lax.bitcast_convert_type(due, jnp.int32), due)
      if s == count - 1:
        attend_in_rounds(qk, row_max, s)
      else:
        denoms[s] = attend(qk, row_max, s)

      size = min(WBATCH, count - batch * WBATCH)
      if final and batch == n_batches - 1:
        copy_o_head(base, batch, pos).start()
      elif pos == size - 1:
        copy_o(base, batch, size).start()

      @_when(head + GROUP < nheads)
      def _():
        copy_v(head + GROUP, s).start()

      next_slot = s + 1 if s + 1 < count else 0

      @_when(head + 1 < nheads)
      def _():
        copy_q(head + 1, next_slot).wait()
        copy_k(head + 1, next_slot).wait()

  for s in range(GROUP):
    copy_q(s, s).start()
    copy_k(s, s).start()
    copy_v(s, s).start()
  copy_q(0, 0).wait()
  copy_k(0, 0).wait()

  def body(t, carry):
    run_heads(t * GROUP, GROUP, final=False)
    return carry

  lax.fori_loop(0, niters, body, 0)

  sizes = list(full_sizes)
  if leftover:
    run_heads(niters * GROUP, leftover, final=True)
    for j in range(-(-leftover // WBATCH)):
      sizes[j] = min(WBATCH, leftover - j * WBATCH)
  for j in range(n_obuf):
    copy_o(0, j, sizes[j]).wait()


@jax.jit
def pallas_standalone__mha_softmax__near_ridge_kernel(
    q: jax.Array,
    k: jax.Array,
    v: jax.Array,
):
  batch, heads, seq_q, dim = q.shape
  seq_k = k.shape[2]
  nheads = batch * heads
  n_obuf = -(-GROUP // WBATCH)

  scratch = (
      [pltpu.VMEM((seq_q, dim), q.dtype)] * GROUP
      + [pltpu.VMEM((seq_k, dim), k.dtype)] * GROUP
      + [pltpu.VMEM((seq_k, dim), v.dtype)] * GROUP
      + [pltpu.VMEM((WBATCH, seq_q, dim), q.dtype)] * n_obuf
      + [pltpu.SemaphoreType.DMA((3, GROUP)), pltpu.SemaphoreType.DMA((n_obuf,))])

  out = pl.pallas_call(
      _kernel,
      in_specs=[pl.BlockSpec(memory_space=pl.ANY)] * 3,
      out_specs=pl.BlockSpec(memory_space=pl.ANY),
      out_shape=jax.ShapeDtypeStruct((nheads, seq_q, dim), q.dtype),
      scratch_shapes=scratch,
      compiler_params=pltpu.CompilerParams(
          vmem_limit_bytes=VMEM_LIMIT,
          disable_bounds_checks=True,
          disable_semaphore_checks=True,
          flags={"XLA_TPU_RESCHEDULE_DMA_DONES": True},
      ),
  )(q.reshape(nheads, seq_q, dim),
    k.reshape(nheads, seq_k, dim),
    v.reshape(nheads, seq_k, dim))

  return out.reshape(batch, heads, seq_q, dim)
```

```python
import jax
import jax.numpy as jnp
from jax import lax
from jax.experimental import pallas as pl
from jax.experimental.pallas import tpu as pltpu

LOG2E = 1.4426950408889634
QK_CONTRACT = (((1,), (1,)), ((), ()))

GROUP = 23
WBATCH = 4
ROUNDS = 4
TIE_LAG = 2
VMEM_LIMIT = 64 * 1024 * 1024


def _batch_sizes():
  return [min(WBATCH, GROUP - first) for first in range(0, GROUP, WBATCH)]


def _bits(ref):
  return ref.bitcast(jnp.int32)


def _as_bf16(words):
  return pltpu.bitcast(words, jnp.bfloat16)


def _after(value, marker_bits, marker):
  return jnp.where(marker_bits != 0, value, marker)


def _when(condition):
  if isinstance(condition, bool):
    return lambda f: f() if condition else None
  return pl.when(condition)


def _kernel(q_hbm, k_hbm, v_hbm, o_hbm, *scratch):
  nheads, _, dim = q_hbm.shape
  seq_k = k_hbm.shape[1]
  niters, leftover = divmod(nheads, GROUP)
  batch_sizes = _batch_sizes()
  n_obuf = len(batch_sizes)
  scale = LOG2E * (dim ** -0.5)

  qbuf = scratch[0:GROUP]
  kbuf = scratch[GROUP:2 * GROUP]
  vbuf = scratch[2 * GROUP:3 * GROUP]
  obuf = scratch[3 * GROUP:3 * GROUP + n_obuf]
  tail_obuf = scratch[3 * GROUP + n_obuf:3 * GROUP + n_obuf + leftover]
  sems, osems = scratch[3 * GROUP + n_obuf + leftover:]

  def copy_q(h, s):
    return pltpu.make_async_copy(q_hbm.at[h], qbuf[s], sems.at[0, s])

  def copy_k(h, s):
    return pltpu.make_async_copy(k_hbm.at[h], kbuf[s], sems.at[1, s])

  def copy_v(h, s):
    return pltpu.make_async_copy(v_hbm.at[h], vbuf[s], sems.at[2, s])

  def copy_o(base, j):
    return pltpu.make_async_copy(
        obuf[j], o_hbm.at[pl.ds(base + j * WBATCH, batch_sizes[j])], osems.at[j])

  def copy_o_tail(i):
    return pltpu.make_async_copy(
        tail_obuf[i], o_hbm.at[niters * GROUP + i], osems.at[n_obuf + i])

  def scores(s):
    qk = lax.dot_general(_as_bf16(_bits(qbuf[s])[...]), _as_bf16(_bits(kbuf[s])[...]),
                         QK_CONTRACT, preferred_element_type=jnp.float32)
    return qk, jnp.max(qk, axis=-1, keepdims=True)

  def store_normalized(acc, denom, out_ref):
    inv = pl.reciprocal(denom, approx=True)
    inv = inv * (2.0 - denom * inv)
    out_ref[...] = (acc * inv).astype(out_ref.dtype)

  def attend(qk, row_max, s, out_ref):
    p = jnp.exp2((qk - row_max) * scale)
    acc = jnp.dot(p.astype(jnp.bfloat16), _as_bf16(_bits(vbuf[s])[...]),
                  preferred_element_type=jnp.float32)
    denom = jnp.sum(p, axis=-1, keepdims=True)
    store_normalized(acc, denom, out_ref)
    return denom

  def attend_in_rounds(qk, row_max, s, out_ref):
    width = seq_k // ROUNDS
    acc = lane_sums = part_acc = part_sum = None
    for r in range(ROUNDS):
      shift = row_max
      if r > 0:
        marker = (lax.bitcast_convert_type(part_acc, jnp.int32)
                  | lax.bitcast_convert_type(part_sum, jnp.int32) | 1)
        shift = _after(jnp.broadcast_to(row_max, part_acc.shape), marker, part_acc)
        shift = jnp.concatenate([shift] * (width // 128), axis=1)
      p = jnp.exp2((qk[:, r * width:(r + 1) * width] - shift) * scale)
      v = _as_bf16(_bits(vbuf[s])[r * width // 2:(r + 1) * width // 2, :])
      part_acc = jnp.dot(p.astype(jnp.bfloat16), v, preferred_element_type=jnp.float32)
      part_sum = p[:, 0:128]
      for j in range(1, width // 128):
        part_sum = part_sum + p[:, 128 * j:128 * (j + 1)]
      acc = part_acc if acc is None else acc + part_acc
      lane_sums = part_sum if lane_sums is None else lane_sums + part_sum
    store_normalized(acc, jnp.sum(lane_sums, axis=-1, keepdims=True), out_ref)

  def run_heads(base, count, after_loop):
    denoms = {}
    for s in range(count):
      head = base + s
      batch, pos = divmod(s, WBATCH)
      out_ref = tail_obuf[s] if after_loop else obuf[batch].at[pos]
      qk, row_max = scores(s)

      @_when(head + GROUP < nheads)
      def _():
        copy_q(head + GROUP, s).start()
        copy_k(head + GROUP, s).start()

      copy_v(head, s).wait()

      if pos == 0 and not after_loop:
        @_when(base > 0)
        def _():
          copy_o(base - GROUP, batch).wait()

      if s >= TIE_LAG:
        due = denoms[s - TIE_LAG]
        row_max = _after(row_max, lax.bitcast_convert_type(due, jnp.int32), due)
      if s == count - 1:
        attend_in_rounds(qk, row_max, s, out_ref)
      else:
        denoms[s] = attend(qk, row_max, s, out_ref)

      if after_loop:
        copy_o_tail(s).start()
      elif pos == batch_sizes[batch] - 1:
        copy_o(base, batch).start()

      @_when(head + GROUP < nheads)
      def _():
        copy_v(head + GROUP, s).start()

      next_slot = s + 1 if s + 1 < count else 0

      @_when(head + 1 < nheads)
      def _():
        copy_q(head + 1, next_slot).wait()
        copy_k(head + 1, next_slot).wait()

  for s in range(GROUP):
    copy_q(s, s).start()
    copy_k(s, s).start()
    copy_v(s, s).start()
  copy_q(0, 0).wait()
  copy_k(0, 0).wait()

  def body(t, carry):
    run_heads(t * GROUP, GROUP, after_loop=False)
    return carry

  lax.fori_loop(0, niters, body, 0)
  run_heads(niters * GROUP, leftover, after_loop=True)

  for j in range(n_obuf):
    copy_o((niters - 1) * GROUP, j).wait()
  for i in range(leftover):
    copy_o_tail(i).wait()


@jax.jit
def pallas_standalone__mha_softmax__near_ridge_kernel(
    q: jax.Array,
    k: jax.Array,
    v: jax.Array,
):
  batch, heads, seq_q, dim = q.shape
  seq_k = k.shape[2]
  nheads = batch * heads
  leftover = nheads % GROUP
  batch_sizes = _batch_sizes()

  scratch = (
      [pltpu.VMEM((seq_q, dim), q.dtype)] * GROUP
      + [pltpu.VMEM((seq_k, dim), k.dtype)] * GROUP
      + [pltpu.VMEM((seq_k, dim), v.dtype)] * GROUP
      + [pltpu.VMEM((n, seq_q, dim), q.dtype) for n in batch_sizes]
      + [pltpu.VMEM((seq_q, dim), q.dtype)] * leftover
      + [pltpu.SemaphoreType.DMA((3, GROUP)),
         pltpu.SemaphoreType.DMA((len(batch_sizes) + leftover,))])

  out = pl.pallas_call(
      _kernel,
      in_specs=[pl.BlockSpec(memory_space=pl.ANY)] * 3,
      out_specs=pl.BlockSpec(memory_space=pl.ANY),
      out_shape=jax.ShapeDtypeStruct((nheads, seq_q, dim), q.dtype),
      scratch_shapes=scratch,
      compiler_params=pltpu.CompilerParams(
          vmem_limit_bytes=VMEM_LIMIT,
          disable_bounds_checks=True,
          disable_semaphore_checks=True,
          flags={"XLA_TPU_RESCHEDULE_DMA_DONES": True},
      ),
  )(q.reshape(nheads, seq_q, dim),
    k.reshape(nheads, seq_k, dim),
    v.reshape(nheads, seq_k, dim))

  return out.reshape(batch, heads, seq_q, dim)
```

```python
import jax
import jax.numpy as jnp
from jax import lax
from jax.experimental import pallas as pl
from jax.experimental.pallas import tpu as pltpu

LOG2E = 1.4426950408889634
QK_CONTRACT = (((1,), (1,)), ((), ()))

GROUP = 23
WBATCH = 4
ROUNDS = 4
TIE_LAG = 2
VMEM_LIMIT = 64 * 1024 * 1024


def _batch_sizes():
  return [min(WBATCH, GROUP - first) for first in range(0, GROUP, WBATCH)]


def _bits(ref):
  return ref.bitcast(jnp.int32)


def _as_bf16(words):
  return pltpu.bitcast(words, jnp.bfloat16)


def _after(value, marker_bits, marker):
  return jnp.where(marker_bits != 0, value, marker)


def _when(condition):
  if isinstance(condition, bool):
    return lambda f: f() if condition else None
  return pl.when(condition)


def _kernel(q_hbm, k_hbm, v_hbm, o_hbm, *scratch):
  nheads, seq_q, dim = q_hbm.shape
  seq_k = k_hbm.shape[1]
  niters, leftover = divmod(nheads, GROUP)
  batch_sizes = _batch_sizes()
  n_obuf = len(batch_sizes)
  scale = LOG2E * (dim ** -0.5)

  qkbuf = scratch[0:GROUP]
  vbuf = scratch[GROUP:2 * GROUP]
  obuf = scratch[2 * GROUP:2 * GROUP + n_obuf]
  tail_obuf = scratch[2 * GROUP + n_obuf:2 * GROUP + n_obuf + leftover]
  sems, osems = scratch[2 * GROUP + n_obuf + leftover:]

  def start_qk(h, s):
    pltpu.make_async_copy(q_hbm.at[h], qkbuf[s].at[pl.ds(0, seq_q)], sems.at[0, s]).start()
    pltpu.make_async_copy(k_hbm.at[h], qkbuf[s].at[pl.ds(seq_q, seq_k)], sems.at[0, s]).start()

  def wait_qk(s):
    pltpu.make_async_copy(qkbuf[s], qkbuf[s], sems.at[0, s]).wait()

  def copy_v(h, s):
    return pltpu.make_async_copy(v_hbm.at[h], vbuf[s], sems.at[1, s])

  def copy_o(base, j):
    return pltpu.make_async_copy(
        obuf[j], o_hbm.at[pl.ds(base + j * WBATCH, batch_sizes[j])], osems.at[j])

  def copy_o_tail(i):
    return pltpu.make_async_copy(
        tail_obuf[i], o_hbm.at[niters * GROUP + i], osems.at[n_obuf + i])

  def scores(s):
    words = _bits(qkbuf[s])
    qk = lax.dot_general(_as_bf16(words[0:seq_q // 2, :]), _as_bf16(words[seq_q // 2:, :]),
                         QK_CONTRACT, preferred_element_type=jnp.float32)
    return qk, jnp.max(qk, axis=-1, keepdims=True)

  def store_normalized(acc, denom, out_ref):
    inv = pl.reciprocal(denom, approx=True)
    inv = inv * (2.0 - denom * inv)
    out_ref[...] = (acc * inv).astype(out_ref.dtype)

  def attend(qk, row_max, s, out_ref):
    p = jnp.exp2((qk - row_max) * scale)
    acc = jnp.dot(p.astype(jnp.bfloat16), _as_bf16(_bits(vbuf[s])[...]),
                  preferred_element_type=jnp.float32)
    denom = jnp.sum(p, axis=-1, keepdims=True)
    store_normalized(acc, denom, out_ref)
    return denom

  def attend_in_rounds(qk, row_max, s, out_ref):
    width = seq_k // ROUNDS
    acc = lane_sums = part_acc = part_sum = None
    for r in range(ROUNDS):
      shift = row_max
      if r > 0:
        marker = (lax.bitcast_convert_type(part_acc, jnp.int32)
                  | lax.bitcast_convert_type(part_sum, jnp.int32) | 1)
        shift = _after(jnp.broadcast_to(row_max, part_acc.shape), marker, part_acc)
        shift = jnp.concatenate([shift] * (width // 128), axis=1)
      p = jnp.exp2((qk[:, r * width:(r + 1) * width] - shift) * scale)
      v = _as_bf16(_bits(vbuf[s])[r * width // 2:(r + 1) * width // 2, :])
      part_acc = jnp.dot(p.astype(jnp.bfloat16), v, preferred_element_type=jnp.float32)
      part_sum = p[:, 0:128]
      for j in range(1, width // 128):
        part_sum = part_sum + p[:, 128 * j:128 * (j + 1)]
      acc = part_acc if acc is None else acc + part_acc
      lane_sums = part_sum if lane_sums is None else lane_sums + part_sum
    store_normalized(acc, jnp.sum(lane_sums, axis=-1, keepdims=True), out_ref)

  def run_heads(base, count, after_loop):
    denoms = {}
    for s in range(count):
      head = base + s
      batch, pos = divmod(s, WBATCH)
      out_ref = tail_obuf[s] if after_loop else obuf[batch].at[pos]
      qk, row_max = scores(s)

      @_when(head + GROUP < nheads)
      def _():
        start_qk(head + GROUP, s)

      copy_v(head, s).wait()

      if pos == 0 and not after_loop:
        @_when(base > 0)
        def _():
          copy_o(base - GROUP, batch).wait()

      if s >= TIE_LAG:
        due = denoms[s - TIE_LAG]
        row_max = _after(row_max, lax.bitcast_convert_type(due, jnp.int32), due)
      if s == count - 1:
        attend_in_rounds(qk, row_max, s, out_ref)
      else:
        denoms[s] = attend(qk, row_max, s, out_ref)

      if after_loop:
        copy_o_tail(s).start()
      elif pos == batch_sizes[batch] - 1:
        copy_o(base, batch).start()

      @_when(head + GROUP < nheads)
      def _():
        copy_v(head + GROUP, s).start()

      next_slot = s + 1 if s + 1 < count else 0

      @_when(head + 1 < nheads)
      def _():
        wait_qk(next_slot)

  for s in range(GROUP):
    start_qk(s, s)
    copy_v(s, s).start()
  wait_qk(0)

  def body(t, carry):
    run_heads(t * GROUP, GROUP, after_loop=False)
    return carry

  lax.fori_loop(0, niters, body, 0)
  run_heads(niters * GROUP, leftover, after_loop=True)

  for j in range(n_obuf):
    copy_o((niters - 1) * GROUP, j).wait()
  for i in range(leftover):
    copy_o_tail(i).wait()


@jax.jit
def pallas_standalone__mha_softmax__near_ridge_kernel(
    q: jax.Array,
    k: jax.Array,
    v: jax.Array,
):
  batch, heads, seq_q, dim = q.shape
  seq_k = k.shape[2]
  nheads = batch * heads
  leftover = nheads % GROUP
  batch_sizes = _batch_sizes()

  scratch = (
      [pltpu.VMEM((seq_q + seq_k, dim), q.dtype)] * GROUP
      + [pltpu.VMEM((seq_k, dim), v.dtype)] * GROUP
      + [pltpu.VMEM((n, seq_q, dim), q.dtype) for n in batch_sizes]
      + [pltpu.VMEM((seq_q, dim), q.dtype)] * leftover
      + [pltpu.SemaphoreType.DMA((2, GROUP)),
         pltpu.SemaphoreType.DMA((len(batch_sizes) + leftover,))])

  out = pl.pallas_call(
      _kernel,
      in_specs=[pl.BlockSpec(memory_space=pl.ANY)] * 3,
      out_specs=pl.BlockSpec(memory_space=pl.ANY),
      out_shape=jax.ShapeDtypeStruct((nheads, seq_q, dim), q.dtype),
      scratch_shapes=scratch,
      compiler_params=pltpu.CompilerParams(
          vmem_limit_bytes=VMEM_LIMIT,
          disable_bounds_checks=True,
          disable_semaphore_checks=True,
          flags={"XLA_TPU_RESCHEDULE_DMA_DONES": True},
      ),
  )(q.reshape(nheads, seq_q, dim),
    k.reshape(nheads, seq_k, dim),
    v.reshape(nheads, seq_k, dim))

  return out.reshape(batch, heads, seq_q, dim)
```

```python
import jax
import jax.numpy as jnp
from jax import lax
from jax.experimental import pallas as pl
from jax.experimental.pallas import tpu as pltpu

LOG2E = 1.4426950408889634
QK_CONTRACT = (((1,), (1,)), ((), ()))

GROUP = 23
WBATCH = 4
ROUNDS = 4
TIE_LAG = 2
VMEM_LIMIT = 64 * 1024 * 1024


def _batch_sizes():
  return [min(WBATCH, GROUP - first) for first in range(0, GROUP, WBATCH)]


def _bits(ref):
  return ref.bitcast(jnp.int32)


def _as_bf16(words):
  return pltpu.bitcast(words, jnp.bfloat16)


def _after(value, marker_bits, marker):
  return jnp.where(marker_bits != 0, value, marker)


def _when(condition):
  if isinstance(condition, bool):
    return lambda f: f() if condition else None
  return pl.when(condition)


def _kernel(q_hbm, k_hbm, v_hbm, o_hbm, *scratch):
  nheads, seq_q, dim = q_hbm.shape
  seq_k = k_hbm.shape[1]
  niters, leftover = divmod(nheads, GROUP)
  batch_sizes = _batch_sizes()
  n_obuf = len(batch_sizes)
  scale = LOG2E * (dim ** -0.5)

  qkbuf = scratch[0:GROUP]
  vbuf = scratch[GROUP:2 * GROUP]
  obuf = scratch[2 * GROUP:2 * GROUP + n_obuf]
  tail_obuf = scratch[2 * GROUP + n_obuf:2 * GROUP + n_obuf + leftover]
  sems, osems = scratch[2 * GROUP + n_obuf + leftover:]

  def start_qk(h, s):
    pltpu.make_async_copy(q_hbm.at[h], qkbuf[s].at[pl.ds(0, seq_q)], sems.at[0, s]).start()
    pltpu.make_async_copy(k_hbm.at[h], qkbuf[s].at[pl.ds(seq_q, seq_k)], sems.at[0, s]).start()

  def wait_qk(s):
    pltpu.make_async_copy(qkbuf[s], qkbuf[s], sems.at[0, s]).wait()

  def copy_v(h, s):
    return pltpu.make_async_copy(v_hbm.at[h], vbuf[s], sems.at[1, s])

  def copy_o(base, j):
    return pltpu.make_async_copy(
        obuf[j], o_hbm.at[pl.ds(base + j * WBATCH, batch_sizes[j])], osems.at[j])

  def copy_o_tail(i):
    return pltpu.make_async_copy(
        tail_obuf[i], o_hbm.at[niters * GROUP + i], osems.at[n_obuf + i])

  def scores(s):
    words = _bits(qkbuf[s])
    qk = lax.dot_general(_as_bf16(words[0:seq_q // 2, :]), _as_bf16(words[seq_q // 2:, :]),
                         QK_CONTRACT, preferred_element_type=jnp.float32)
    return qk, jnp.max(qk, axis=-1, keepdims=True)

  def store_normalized(acc, denom, out_ref):
    inv = pl.reciprocal(denom, approx=True)
    inv = inv * (2.0 - denom * inv)
    out_ref[...] = (acc * inv).astype(out_ref.dtype)

  def attend(qk, row_max, s, out_ref):
    p = jnp.exp2((qk - row_max) * scale)
    acc = jnp.dot(p.astype(jnp.bfloat16), _as_bf16(_bits(vbuf[s])[...]),
                  preferred_element_type=jnp.float32)
    denom = jnp.sum(p, axis=-1, keepdims=True)
    store_normalized(acc, denom, out_ref)
    return denom

  def attend_in_rounds(qk, row_max, s, out_ref):
    width = seq_k // ROUNDS
    acc = lane_sums = part_acc = part_sum = None
    for r in range(ROUNDS):
      shift = row_max
      if r > 0:
        marker = (lax.bitcast_convert_type(part_acc, jnp.int32)
                  | lax.bitcast_convert_type(part_sum, jnp.int32) | 1)
        shift = _after(jnp.broadcast_to(row_max, part_acc.shape), marker, part_acc)
        shift = jnp.concatenate([shift] * (width // 128), axis=1)
      p = jnp.exp2((qk[:, r * width:(r + 1) * width] - shift) * scale)
      v = _as_bf16(_bits(vbuf[s])[r * width // 2:(r + 1) * width // 2, :])
      part_acc = jnp.dot(p.astype(jnp.bfloat16), v, preferred_element_type=jnp.float32)
      part_sum = p[:, 0:128]
      for j in range(1, width // 128):
        part_sum = part_sum + p[:, 128 * j:128 * (j + 1)]
      acc = part_acc if acc is None else acc + part_acc
      lane_sums = part_sum if lane_sums is None else lane_sums + part_sum
    store_normalized(acc, jnp.sum(lane_sums, axis=-1, keepdims=True), out_ref)

  def run_heads(base, count, after_loop):
    denoms = {}
    for s in range(count):
      head = base + s
      batch, pos = divmod(s, WBATCH)
      out_ref = tail_obuf[s] if after_loop else obuf[batch].at[pos]
      qk, row_max = scores(s)

      def refill_qk():
        @_when(head + GROUP < nheads)
        def _():
          start_qk(head + GROUP, s)

      if s == 0:
        refill_qk()
      copy_v(head, s).wait()

      if pos == 0 and not after_loop:
        @_when(base > 0)
        def _():
          copy_o(base - GROUP, batch).wait()

      if s > 0:
        refill_qk()

      if s >= TIE_LAG:
        due = denoms[s - TIE_LAG]
        row_max = _after(row_max, lax.bitcast_convert_type(due, jnp.int32), due)
      if s == count - 1:
        attend_in_rounds(qk, row_max, s, out_ref)
      else:
        denoms[s] = attend(qk, row_max, s, out_ref)

      if after_loop:
        copy_o_tail(s).start()
      elif pos == batch_sizes[batch] - 1:
        copy_o(base, batch).start()

      @_when(head + GROUP < nheads)
      def _():
        copy_v(head + GROUP, s).start()

      next_slot = s + 1 if s + 1 < count else 0

      @_when(head + 1 < nheads)
      def _():
        wait_qk(next_slot)

  for s in range(GROUP):
    start_qk(s, s)
    copy_v(s, s).start()
  wait_qk(0)

  def body(t, carry):
    run_heads(t * GROUP, GROUP, after_loop=False)
    return carry

  lax.fori_loop(0, niters, body, 0)
  run_heads(niters * GROUP, leftover, after_loop=True)

  for j in range(n_obuf):
    copy_o((niters - 1) * GROUP, j).wait()
  for i in range(leftover):
    copy_o_tail(i).wait()


@jax.jit
def pallas_standalone__mha_softmax__near_ridge_kernel(
    q: jax.Array,
    k: jax.Array,
    v: jax.Array,
):
  batch, heads, seq_q, dim = q.shape
  seq_k = k.shape[2]
  nheads = batch * heads
  leftover = nheads % GROUP
  batch_sizes = _batch_sizes()

  scratch = (
      [pltpu.VMEM((seq_q + seq_k, dim), q.dtype)] * GROUP
      + [pltpu.VMEM((seq_k, dim), v.dtype)] * GROUP
      + [pltpu.VMEM((n, seq_q, dim), q.dtype) for n in batch_sizes]
      + [pltpu.VMEM((seq_q, dim), q.dtype)] * leftover
      + [pltpu.SemaphoreType.DMA((2, GROUP)),
         pltpu.SemaphoreType.DMA((len(batch_sizes) + leftover,))])

  out = pl.pallas_call(
      _kernel,
      in_specs=[pl.BlockSpec(memory_space=pl.ANY)] * 3,
      out_specs=pl.BlockSpec(memory_space=pl.ANY),
      out_shape=jax.ShapeDtypeStruct((nheads, seq_q, dim), q.dtype),
      scratch_shapes=scratch,
      compiler_params=pltpu.CompilerParams(
          vmem_limit_bytes=VMEM_LIMIT,
          disable_bounds_checks=True,
          disable_semaphore_checks=True,
          flags={"XLA_TPU_RESCHEDULE_DMA_DONES": True},
      ),
  )(q.reshape(nheads, seq_q, dim),
    k.reshape(nheads, seq_k, dim),
    v.reshape(nheads, seq_k, dim))

  return out.reshape(batch, heads, seq_q, dim)
```

```python
import jax
import jax.numpy as jnp
from jax import lax
from jax.experimental import pallas as pl
from jax.experimental.pallas import tpu as pltpu

LOG2E = 1.4426950408889634
QK_CONTRACT = (((1,), (1,)), ((), ()))

GROUP = 23
WBATCH = 4
ROUNDS = 4
TIE_LAG = 2
HOLD = 3
VMEM_LIMIT = 64 * 1024 * 1024


def _batch_sizes():
  return [min(WBATCH, GROUP - first) for first in range(0, GROUP, WBATCH)]


def _bits(ref):
  return ref.bitcast(jnp.int32)


def _as_bf16(words):
  return pltpu.bitcast(words, jnp.bfloat16)


def _after(value, marker_bits, marker):
  return jnp.where(marker_bits != 0, value, marker)


def _when(condition):
  if isinstance(condition, bool):
    return lambda f: f() if condition else None
  return pl.when(condition)


def _kernel(q_hbm, k_hbm, v_hbm, o_hbm, *scratch):
  nheads, seq_q, dim = q_hbm.shape
  seq_k = k_hbm.shape[1]
  niters, leftover = divmod(nheads, GROUP)
  batch_sizes = _batch_sizes()
  n_obuf = len(batch_sizes)
  scale = LOG2E * (dim ** -0.5)

  qkbuf = scratch[0:GROUP]
  vbuf = scratch[GROUP:2 * GROUP]
  obuf = scratch[2 * GROUP:2 * GROUP + n_obuf]
  tail_obuf = scratch[2 * GROUP + n_obuf:2 * GROUP + n_obuf + leftover]
  sems, osems = scratch[2 * GROUP + n_obuf + leftover:]

  def start_qk(h, s):
    pltpu.make_async_copy(q_hbm.at[h], qkbuf[s].at[pl.ds(0, seq_q)], sems.at[0, s]).start()
    pltpu.make_async_copy(k_hbm.at[h], qkbuf[s].at[pl.ds(seq_q, seq_k)], sems.at[0, s]).start()

  def wait_qk(s):
    pltpu.make_async_copy(qkbuf[s], qkbuf[s], sems.at[0, s]).wait()

  def copy_v(h, s):
    return pltpu.make_async_copy(v_hbm.at[h], vbuf[s], sems.at[1, s])

  def copy_o(base, j):
    return pltpu.make_async_copy(
        obuf[j], o_hbm.at[pl.ds(base + j * WBATCH, batch_sizes[j])], osems.at[j])

  def copy_o_tail(i):
    return pltpu.make_async_copy(
        tail_obuf[i], o_hbm.at[niters * GROUP + i], osems.at[n_obuf + i])

  def scores(s):
    words = _bits(qkbuf[s])
    qk = lax.dot_general(_as_bf16(words[0:seq_q // 2, :]), _as_bf16(words[seq_q // 2:, :]),
                         QK_CONTRACT, preferred_element_type=jnp.float32)
    return qk, jnp.max(qk, axis=-1, keepdims=True)

  def store_normalized(acc, denom, out_ref):
    inv = pl.reciprocal(denom, approx=True)
    inv = inv * (2.0 - denom * inv)
    out_ref[...] = (acc * inv).astype(out_ref.dtype)

  def attend(qk, row_max, s):
    p = jnp.exp2((qk - row_max) * scale)
    acc = jnp.dot(p.astype(jnp.bfloat16), _as_bf16(_bits(vbuf[s])[...]),
                  preferred_element_type=jnp.float32)
    return acc, jnp.sum(p, axis=-1, keepdims=True)

  def attend_in_rounds(qk, row_max, s):
    width = seq_k // ROUNDS
    acc = lane_sums = part_acc = part_sum = None
    for r in range(ROUNDS):
      shift = row_max
      if r > 0:
        marker = (lax.bitcast_convert_type(part_acc, jnp.int32)
                  | lax.bitcast_convert_type(part_sum, jnp.int32) | 1)
        shift = _after(jnp.broadcast_to(row_max, part_acc.shape), marker, part_acc)
        shift = jnp.concatenate([shift] * (width // 128), axis=1)
      p = jnp.exp2((qk[:, r * width:(r + 1) * width] - shift) * scale)
      v = _as_bf16(_bits(vbuf[s])[r * width // 2:(r + 1) * width // 2, :])
      part_acc = jnp.dot(p.astype(jnp.bfloat16), v, preferred_element_type=jnp.float32)
      part_sum = p[:, 0:128]
      for j in range(1, width // 128):
        part_sum = part_sum + p[:, 128 * j:128 * (j + 1)]
      acc = part_acc if acc is None else acc + part_acc
      lane_sums = part_sum if lane_sums is None else lane_sums + part_sum
    return acc, jnp.sum(lane_sums, axis=-1, keepdims=True)

  def run_heads(base, count, after_loop):
    results = {}

    def finish(s, denom):
      batch, pos = divmod(s, WBATCH)
      if after_loop:
        store_normalized(results[s][0], denom, tail_obuf[s])
        copy_o_tail(s).start()
      else:
        store_normalized(results[s][0], denom, obuf[batch].at[pos])
        if pos == batch_sizes[batch] - 1:
          copy_o(base, batch).start()

    for s in range(count):
      head = base + s
      batch, pos = divmod(s, WBATCH)
      qk, row_max = scores(s)

      def refill_qk():
        @_when(head + GROUP < nheads)
        def _():
          start_qk(head + GROUP, s)

      if s == 0:
        refill_qk()
      copy_v(head, s).wait()

      if pos == 0 and not after_loop:
        @_when(base > 0)
        def _():
          copy_o(base - GROUP, batch).wait()

      if s > 0:
        refill_qk()

      if s >= HOLD:
        denom = results[s - HOLD][1]
        cue = qk[:, 256:384]
        finish(s - HOLD, _after(jnp.broadcast_to(denom, cue.shape),
                                lax.bitcast_convert_type(cue, jnp.int32) | 1, cue))
      if s >= TIE_LAG:
        due = results[s - TIE_LAG][1]
        row_max = _after(row_max, lax.bitcast_convert_type(due, jnp.int32), due)

      results[s] = (attend_in_rounds if s == count - 1 else attend)(qk, row_max, s)
      if s + HOLD >= count:
        finish(s, results[s][1])

      @_when(head + GROUP < nheads)
      def _():
        copy_v(head + GROUP, s).start()

      next_slot = s + 1 if s + 1 < count else 0

      @_when(head + 1 < nheads)
      def _():
        wait_qk(next_slot)

  for s in range(GROUP):
    start_qk(s, s)
    copy_v(s, s).start()
  wait_qk(0)

  def body(t, carry):
    run_heads(t * GROUP, GROUP, after_loop=False)
    return carry

  lax.fori_loop(0, niters, body, 0)
  run_heads(niters * GROUP, leftover, after_loop=True)

  for j in range(n_obuf):
    copy_o((niters - 1) * GROUP, j).wait()
  for i in range(leftover):
    copy_o_tail(i).wait()


@jax.jit
def pallas_standalone__mha_softmax__near_ridge_kernel(
    q: jax.Array,
    k: jax.Array,
    v: jax.Array,
):
  batch, heads, seq_q, dim = q.shape
  seq_k = k.shape[2]
  nheads = batch * heads
  leftover = nheads % GROUP
  batch_sizes = _batch_sizes()

  scratch = (
      [pltpu.VMEM((seq_q + seq_k, dim), q.dtype)] * GROUP
      + [pltpu.VMEM((seq_k, dim), v.dtype)] * GROUP
      + [pltpu.VMEM((n, seq_q, dim), q.dtype) for n in batch_sizes]
      + [pltpu.VMEM((seq_q, dim), q.dtype)] * leftover
      + [pltpu.SemaphoreType.DMA((2, GROUP)),
         pltpu.SemaphoreType.DMA((len(batch_sizes) + leftover,))])

  out = pl.pallas_call(
      _kernel,
      in_specs=[pl.BlockSpec(memory_space=pl.ANY)] * 3,
      out_specs=pl.BlockSpec(memory_space=pl.ANY),
      out_shape=jax.ShapeDtypeStruct((nheads, seq_q, dim), q.dtype),
      scratch_shapes=scratch,
      compiler_params=pltpu.CompilerParams(
          vmem_limit_bytes=VMEM_LIMIT,
          disable_bounds_checks=True,
          disable_semaphore_checks=True,
          flags={"XLA_TPU_RESCHEDULE_DMA_DONES": True},
      ),
  )(q.reshape(nheads, seq_q, dim),
    k.reshape(nheads, seq_k, dim),
    v.reshape(nheads, seq_k, dim))

  return out.reshape(batch, heads, seq_q, dim)
```

```python
import jax
import jax.numpy as jnp
from jax import lax
from jax.experimental import pallas as pl
from jax.experimental.pallas import tpu as pltpu

LOG2E = 1.4426950408889634
QK_CONTRACT = (((1,), (1,)), ((), ()))

GROUP = 23
WBATCH = 4
ROUNDS = 4
TIE_LAG = 2
HOLD = 3
VMEM_LIMIT = 64 * 1024 * 1024


def _batch_sizes():
  return [min(WBATCH, GROUP - first) for first in range(0, GROUP, WBATCH)]


def _bits(ref):
  return ref.bitcast(jnp.int32)


def _as_bf16(words):
  return pltpu.bitcast(words, jnp.bfloat16)


def _after(value, marker_bits, marker):
  return jnp.where(marker_bits != 0, value, marker)


def _when(condition):
  if isinstance(condition, bool):
    return lambda f: f() if condition else None
  return pl.when(condition)


def _kernel(q_hbm, k_hbm, v_hbm, o_hbm, *scratch):
  nheads, seq_q, dim = q_hbm.shape
  seq_k = k_hbm.shape[1]
  niters, leftover = divmod(nheads, GROUP)
  batch_sizes = _batch_sizes()
  n_obuf = len(batch_sizes)
  scale = LOG2E * (dim ** -0.5)

  qkbuf = scratch[0:GROUP]
  vbuf = scratch[GROUP:2 * GROUP]
  obuf = scratch[2 * GROUP:2 * GROUP + n_obuf]
  tail_obuf = scratch[2 * GROUP + n_obuf:2 * GROUP + n_obuf + leftover]
  held_acc, held_denom, sems, osems = scratch[2 * GROUP + n_obuf + leftover:]
  last_batch = n_obuf - 1
  assert batch_sizes[last_batch] == HOLD and leftover >= HOLD

  def start_qk(h, s):
    pltpu.make_async_copy(q_hbm.at[h], qkbuf[s].at[pl.ds(0, seq_q)], sems.at[0, s]).start()
    pltpu.make_async_copy(k_hbm.at[h], qkbuf[s].at[pl.ds(seq_q, seq_k)], sems.at[0, s]).start()

  def wait_qk(s):
    pltpu.make_async_copy(qkbuf[s], qkbuf[s], sems.at[0, s]).wait()

  def copy_v(h, s):
    return pltpu.make_async_copy(v_hbm.at[h], vbuf[s], sems.at[1, s])

  def copy_o(base, j):
    return pltpu.make_async_copy(
        obuf[j], o_hbm.at[pl.ds(base + j * WBATCH, batch_sizes[j])], osems.at[j])

  def copy_o_tail(i):
    return pltpu.make_async_copy(
        tail_obuf[i], o_hbm.at[niters * GROUP + i], osems.at[n_obuf + i])

  def scores(s):
    words = _bits(qkbuf[s])
    qk = lax.dot_general(_as_bf16(words[0:seq_q // 2, :]), _as_bf16(words[seq_q // 2:, :]),
                         QK_CONTRACT, preferred_element_type=jnp.float32)
    return qk, jnp.max(qk, axis=-1, keepdims=True)

  def store_normalized(acc, denom, out_ref):
    inv = pl.reciprocal(denom, approx=True)
    inv = inv * (2.0 - denom * inv)
    out_ref[...] = (acc * inv).astype(o_hbm.dtype)

  def attend(qk, row_max, s):
    p = jnp.exp2((qk - row_max) * scale)
    acc = jnp.dot(p.astype(jnp.bfloat16), _as_bf16(_bits(vbuf[s])[...]),
                  preferred_element_type=jnp.float32)
    return acc, jnp.sum(p, axis=-1, keepdims=True)

  def attend_in_rounds(qk, row_max, s):
    width = seq_k // ROUNDS
    acc = lane_sums = part_acc = part_sum = None
    for r in range(ROUNDS):
      shift = row_max
      if r > 0:
        marker = (lax.bitcast_convert_type(part_acc, jnp.int32)
                  | lax.bitcast_convert_type(part_sum, jnp.int32) | 1)
        shift = _after(jnp.broadcast_to(row_max, part_acc.shape), marker, part_acc)
        shift = jnp.concatenate([shift] * (width // 128), axis=1)
      p = jnp.exp2((qk[:, r * width:(r + 1) * width] - shift) * scale)
      v = _as_bf16(_bits(vbuf[s])[r * width // 2:(r + 1) * width // 2, :])
      part_acc = jnp.dot(p.astype(jnp.bfloat16), v, preferred_element_type=jnp.float32)
      part_sum = p[:, 0:128]
      for j in range(1, width // 128):
        part_sum = part_sum + p[:, 128 * j:128 * (j + 1)]
      acc = part_acc if acc is None else acc + part_acc
      lane_sums = part_sum if lane_sums is None else lane_sums + part_sum
    return acc, jnp.sum(lane_sums, axis=-1, keepdims=True)

  def run_heads(base, count, after_loop):
    results = {}

    def finish(s, denom):
      batch, pos = divmod(s, WBATCH)
      if after_loop:
        store_normalized(results[s][0], denom, tail_obuf[s])
        copy_o_tail(s).start()
      else:
        store_normalized(results[s][0], denom, obuf[batch].at[pos])
        if pos == batch_sizes[batch] - 1:
          copy_o(base, batch).start()

    for s in range(count):
      head = base + s
      batch, pos = divmod(s, WBATCH)
      qk, row_max = scores(s)

      def refill_qk():
        @_when(head + GROUP < nheads)
        def _():
          start_qk(head + GROUP, s)

      if s == 0:
        refill_qk()
      copy_v(head, s).wait()

      if pos == 0 and not after_loop and batch != last_batch:
        @_when(base > 0)
        def _():
          copy_o(base - GROUP, batch).wait()
      if s == 0:
        @_when(base >= 2 * GROUP)
        def _():
          copy_o(base - 2 * GROUP, last_batch).wait()

      if s > 0:
        refill_qk()

      cue = qk[:, 384:512]
      cue_bits = lax.bitcast_convert_type(cue, jnp.int32) | 1
      if s >= HOLD:
        finish(s - HOLD, _after(jnp.broadcast_to(results[s - HOLD][1], cue.shape),
                                cue_bits, cue))
      else:
        store_normalized(held_acc[s], _after(held_denom[s], cue_bits, cue),
                         obuf[last_batch].at[s])
        if s == HOLD - 1:
          @_when(base > 0)
          def _():
            copy_o(base - GROUP, last_batch).start()

      if s >= TIE_LAG:
        due = results[s - TIE_LAG][1]
        row_max = _after(row_max, lax.bitcast_convert_type(due, jnp.int32), due)

      results[s] = (attend_in_rounds if s == count - 1 else attend)(qk, row_max, s)
      if s + HOLD >= count:
        if after_loop:
          finish(s, results[s][1])
        else:
          held_acc[s + HOLD - count] = results[s][0]
          held_denom[s + HOLD - count] = jnp.broadcast_to(results[s][1], (seq_q, 128))

      @_when(head + GROUP < nheads)
      def _():
        copy_v(head + GROUP, s).start()

      next_slot = s + 1 if s + 1 < count else 0

      @_when(head + 1 < nheads)
      def _():
        wait_qk(next_slot)

  for s in range(GROUP):
    start_qk(s, s)
    copy_v(s, s).start()
  held_acc[...] = jnp.zeros(held_acc.shape, jnp.float32)
  held_denom[...] = jnp.ones(held_denom.shape, jnp.float32)
  wait_qk(0)

  def body(t, carry):
    run_heads(t * GROUP, GROUP, after_loop=False)
    return carry

  lax.fori_loop(0, niters, body, 0)
  run_heads(niters * GROUP, leftover, after_loop=True)

  for j in range(n_obuf):
    copy_o((niters - 1) * GROUP, j).wait()
  for i in range(leftover):
    copy_o_tail(i).wait()


@jax.jit
def pallas_standalone__mha_softmax__near_ridge_kernel(
    q: jax.Array,
    k: jax.Array,
    v: jax.Array,
):
  batch, heads, seq_q, dim = q.shape
  seq_k = k.shape[2]
  nheads = batch * heads
  leftover = nheads % GROUP
  batch_sizes = _batch_sizes()

  scratch = (
      [pltpu.VMEM((seq_q + seq_k, dim), q.dtype)] * GROUP
      + [pltpu.VMEM((seq_k, dim), v.dtype)] * GROUP
      + [pltpu.VMEM((n, seq_q, dim), q.dtype) for n in batch_sizes]
      + [pltpu.VMEM((seq_q, dim), q.dtype)] * leftover
      + [pltpu.VMEM((HOLD, seq_q, dim), jnp.float32), pltpu.VMEM((HOLD, seq_q, 128), jnp.float32)]
      + [pltpu.SemaphoreType.DMA((2, GROUP)),
         pltpu.SemaphoreType.DMA((len(batch_sizes) + leftover,))])

  out = pl.pallas_call(
      _kernel,
      in_specs=[pl.BlockSpec(memory_space=pl.ANY)] * 3,
      out_specs=pl.BlockSpec(memory_space=pl.ANY),
      out_shape=jax.ShapeDtypeStruct((nheads, seq_q, dim), q.dtype),
      scratch_shapes=scratch,
      compiler_params=pltpu.CompilerParams(
          vmem_limit_bytes=VMEM_LIMIT,
          disable_bounds_checks=True,
          disable_semaphore_checks=True,
          flags={"XLA_TPU_RESCHEDULE_DMA_DONES": True},
      ),
  )(q.reshape(nheads, seq_q, dim),
    k.reshape(nheads, seq_k, dim),
    v.reshape(nheads, seq_k, dim))

  return out.reshape(batch, heads, seq_q, dim)
```
